```python
import jax
import jax.numpy as jnp

def _softmax(x, axis=-1):
    return jax.nn.softmax(x, axis=axis)

def _gelu(x):
    return jax.nn.gelu(x, approximate=True)

def _silu(x):
    return jax.nn.silu(x)

def _sigmoid(x):
    return jax.nn.sigmoid(x)

def _layernorm(x, axis=-1, eps=1e-05):
    m = jnp.mean(x, axis=axis, keepdims=True)
    v = jnp.var(x, axis=axis, keepdims=True)
    return (x - m) / jnp.sqrt(v + eps)

def _scatter_add(tgt, idx, src, axis=0):
    return tgt.at[idx].add(src)

def _segment_sum(src, seg, n):
    return jax.ops.segment_sum(src, seg, n)

class _Rng:

    def __init__(self, key):
        self._k = key

    def _next(self):
        self._k, sub = jax.random.split(self._k)
        return sub

    def normal(self, shape):
        return jax.random.normal(self._next(), shape, dtype=jnp.bfloat16)

    def randint(self, lo, hi, shape):
        return jax.random.randint(self._next(), shape, lo, hi, dtype=jnp.int32)

    def uniform(self, shape, lo=0.0, hi=1.0):
        return jax.random.uniform(self._next(), shape, jnp.bfloat16, lo, hi)

    def permutation(self, n):
        return jax.random.permutation(self._next(), n)
kernel_name = 'adaLN_cond__ssm_conv_h3__mixer_s_mlp__prompt'

def setup_inputs():
    _rng = _Rng(jax.random.key(int.from_bytes(__import__("os").urandom(4), "little")))
    _w = lambda a: (lambda t: t.astype(jnp.bfloat16) if jnp.issubdtype(t.dtype, jnp.floating) else t)(jnp.asarray(a))

    def _A_setup():
        B, S, D = (1, 2048, 640)
        ks = 4
        return {'q': _w((lambda *s: _rng.normal(s) * 0.05)(B, S, D)), 'k': _w((lambda *s: _rng.normal(s) * 0.05)(B, S, D)), 'v': _w((lambda *s: _rng.normal(s) * 0.05)(B, S, D)), 'shift_k': _w((lambda *s: _rng.normal(s) * 0.05)(D, ks) * 0.5), 'ssm_k': _w((lambda *s: _rng.normal(s) * 0.05)(D, S) * (1.0 / S ** 0.5)), 'ssm_D': _w((lambda *s: _rng.normal(s) * 0.05)(D))}
    _A_in = _A_setup()

    def _B_setup():
        B, S, D, F = (1, 2048, 640, 1728)
        return {'x': _w((lambda *s: _rng.normal(s) * 0.05)(B, S, D)), 'w1': _w((lambda *s: _rng.normal(s) * 0.05)(D, D) * D ** (-0.5)), 'w2': _w((lambda *s: _rng.normal(s) * 0.05)(D, D) * D ** (-0.5)), 'w3': _w((lambda *s: _rng.normal(s) * 0.05)(D, F) * D ** (-0.5)), 'w4': _w((lambda *s: _rng.normal(s) * 0.05)(F, D) * F ** (-0.5))}
    _B_in = _B_setup()
    return {'A_q': _A_in['q'], 'A_k': _A_in['k'], 'A_v': _A_in['v'], 'A_shift_k': _A_in['shift_k'], 'A_ssm_k': _A_in['ssm_k'], 'A_ssm_D': _A_in['ssm_D'], 'B_x': _B_in['x'], 'B_w1': _B_in['w1'], 'B_w2': _B_in['w2'], 'B_w3': _B_in['w3'], 'B_w4': _B_in['w4'], 'c': _w((lambda *s: _rng.normal(s) * 0.05)(1, 640)), 'w_mod': _w((lambda *s: _rng.normal(s) * 0.05)(640, 6 * 640) * 640 ** (-0.5))}

def reference(A_q, A_k, A_v, A_shift_k, A_ssm_k, A_ssm_D, B_x, B_w1, B_w2, B_w3, B_w4, c, w_mod):

    def _A_ref(q, k, v, shift_k, ssm_k, ssm_D):
        B, S, D = q.shape
        ks = shift_k.shape[-1]
        k_pad = jnp.pad(k, ((0, 0), (ks - 1, 0), (0, 0)))
        k_shift = jnp.zeros_like(k)
        for t in range(ks):
            k_shift = k_shift + k_pad[:, t:t + S, :] * shift_k[:, ks - 1 - t][None, None, :]
        kv = k_shift * v
        L = 2 * S
        kv_pad = jnp.pad(kv, ((0, 0), (0, S), (0, 0)))
        kf_pad = jnp.pad(ssm_k, ((0, 0), (0, S)))
        kv_f = (lambda x, axes=(-2, -1): jnp.fft.rfft2(x.astype(jnp.float32), axes=axes))(kv_pad[:, None, :, :], axes=(1, 2))
        kf_f = (lambda x, axes=(-2, -1): jnp.fft.rfft2(x.astype(jnp.float32), axes=axes))(kf_pad[:, None, :], axes=(1, 2))
        kf_f = (lambda x, *d: x.transpose(*d))(kf_f, 1, 2, 0)
        y_f = kv_f * kf_f[None, :, :, :]
        y = (lambda x, s, axes=(-2, -1): jnp.fft.irfft2(x, s=s, axes=axes).astype(jnp.bfloat16))(y_f, (1, L), axes=(1, 2))[:, 0, :S, :]
        y = y + kv * ssm_D[None, None, :]
        return q * y

    def _B_ref(x, w1, w2, w3, w4):
        B, S, D = x.shape
        h = _gelu(_layernorm(x, axis=-1) @ w1)
        c = D // 4
        g0 = jnp.pad(h[:, :, 0 * c:1 * c], ((0, 0), (1, 0), (0, 0)))[:, :S, :]
        g1 = jnp.pad(h[:, :, 1 * c:2 * c], ((0, 0), (0, 1), (0, 0)))[:, 1:, :]
        g2 = jnp.pad(h[:, :, 2 * c:3 * c], ((0, 0), (2, 0), (0, 0)))[:, :S, :]
        g3 = jnp.pad(h[:, :, 3 * c:], ((0, 0), (0, 2), (0, 0)))[:, 2:, :]
        hs = jnp.concatenate([g0, g1, g2, g3], axis=-1) @ w2
        x1 = x + hs
        h2 = _gelu(_layernorm(x1, axis=-1) @ w3) @ w4
        return x1 + h2
    x = A_q
    mod = (_silu(c) @ w_mod).reshape(c.shape[0], 6, 1, -1)
    sa, ca, ga, sb, cb, gb = (mod[:, 0].copy(), mod[:, 1].copy(), mod[:, 2].copy(), mod[:, 3].copy(), mod[:, 4].copy(), mod[:, 5].copy())
    h = _layernorm(x, axis=-1) * (1 + ca) + sa
    x = x + ga * _A_ref(h, A_k, A_v, A_shift_k, A_ssm_k, A_ssm_D)
    h = _layernorm(x, axis=-1) * (1 + cb) + sb
    x = x + gb * _B_ref(h, B_w1, B_w2, B_w3, B_w4)
    return x
```

```python
import numpy as np
import jax
import jax.numpy as jnp
import jax.experimental.pallas as pl
import jax.experimental.pallas.tpu as pltpu

S, D, F = 2048, 640, 1728
C = 128
NC = S // C
TM = 256
NT = S // TM
EPS = 1e-5
BF, F32 = jnp.bfloat16, jnp.float32


def _dft_mats():
    f = np.concatenate([np.arange(0, C, 2), np.arange(1, C, 2)])
    n = np.arange(C)
    ang = np.pi * (2 * f[:, None] + 1) * n[None, :] / (2 * C)
    re, im = np.cos(ang), -np.sin(ang)
    fwd = np.stack([re.reshape(C // 8, 8, C), im.reshape(C // 8, 8, C)], 1).reshape(2 * C, C)
    inv = fwd.T / C
    return fwd.astype(BF), inv.astype(BF)


_WF, _WI = _dft_mats()


def _ln(x):
    m = jnp.mean(x, axis=-1, keepdims=True)
    xc = x - m
    v = jnp.mean(xc * xc, axis=-1, keepdims=True)
    return xc * jax.lax.rsqrt(v + EPS)


def _gelu(x):
    c0 = float(np.sqrt(2.0 / np.pi))
    t = jnp.tanh(x * (c0 + (c0 * 0.044715) * (x * x)))
    hx = 0.5 * x
    return hx + hx * t


def _dot(a, b):
    return jnp.dot(a, b, preferred_element_type=F32)


def _dot_nt(a, b):
    return jax.lax.dot_general(a, b, (((1,), (1,)), ((), ())), preferred_element_type=F32)


def _kernel(q_h, k_h, v_h, shk_h, ssm_h, ssd_h, w1_h, w2_h, w3_h, w4_h, c_h, wm_h,
            wf_h, wi_h, o_h, shk_ref, ssd_ref, c_ref, wf_ref, wi_ref,
            q_v, k_v, v_v, ssm_v, w1_v, w2_v, w3_v, w4_v, wm_v,
            kf, uf, yf, x2_v, hb_v, hh_v, o_v, sems):
    NJ = D // 128
    cp_ssm = [pltpu.make_async_copy(ssm_h.at[pl.ds(128 * j, 128)], ssm_v.at[pl.ds(128 * j, 128)], sems.at[j])
              for j in range(NJ)]
    NK = 4
    RK = S // NK
    cp_k = [pltpu.make_async_copy(k_h.at[0, pl.ds(RK * j, RK)], k_v.at[pl.ds(16 + RK * j, RK)], sems.at[5 + j])
            for j in range(NK)]
    cp_v = [pltpu.make_async_copy(v_h.at[0, pl.ds(RK * j, RK)], v_v.at[pl.ds(RK * j, RK)], sems.at[9 + j])
            for j in range(NK)]
    cp_wm = pltpu.make_async_copy(wm_h, wm_v, sems.at[13])
    cp_q = pltpu.make_async_copy(q_h.at[0], q_v, sems.at[14])
    cp_w = [pltpu.make_async_copy(a, b, sems.at[15 + i])
            for i, (a, b) in enumerate([(w1_h, w1_v), (w2_h, w2_v), (w3_h, w3_v), (w4_h, w4_v)])]
    cp_s = [pltpu.make_async_copy(a, b, sems.at[20 + i])
            for i, (a, b) in enumerate([(wf_h, wf_ref), (ssd_h, ssd_ref), (shk_h, shk_ref), (c_h, c_ref), (wi_h, wi_ref)])]
    for cp in cp_s:
        cp.start()
    for cp in cp_ssm:
        cp.start()
    cp_k[0].start()
    cp_v[0].start()

    k_v[pl.ds(0, 16), :] = jnp.zeros((16, D), BF)
    hh_v[pl.ds(0, 8), :] = jnp.zeros((8, D), F32)
    hh_v[pl.ds(8 + S, 8), :] = jnp.zeros((8, D), F32)
    for cp in cp_s:
        cp.wait()
    wf = wf_ref[...]
    ssd = ssd_ref[...].astype(F32).reshape(1, D)

    for j in range(NJ):
        cp_ssm[j].wait()
        if j + 1 < NK:
            cp_k[j + 1].start()
            cp_v[j + 1].start()
        if j == NJ - 2:
            cp_wm.start()
        lanes = slice(128 * j, 128 * (j + 1))
        prev = None
        for m in range(NC):
            kh = _dot_nt(wf, ssm_v[lanes, C * m:C * (m + 1)]).reshape(2, C // 16, 2, 8, 128)
            re, im = kh[:, :, 0], kh[:, :, 1]
            if m == 0:
                re = re + ssd[:, lanes]
                ore, oim = re, im
            else:
                pre, pim = prev
                ore = jnp.stack([re[0] - pim[0], re[1] + pim[1]])
                oim = jnp.stack([im[0] + pre[0], im[1] - pre[1]])
            prev = (re, im)
            kf[m, :, lanes] = jnp.stack([ore, oim], axis=2).reshape(2 * C, 128)

    shk = shk_ref[...].astype(F32)
    for b in range(NC):
        if b % (NC // NK) == 0:
            cp_k[b // (NC // NK)].wait()
            cp_v[b // (NC // NK)].wait()
        if b == 4:
            cp_q.start()
            cp_w[0].start()
        kk = k_v[pl.ds(C * b, C + 16), :].astype(F32)
        ks = kk[16:16 + C] * shk[0:1]
        for t in range(1, 4):
            ks = ks + kk[16 - t:16 - t + C] * shk[t:t + 1]
        kv = ks * v_v[pl.ds(C * b, C), :].astype(F32)
        uf[b] = _dot(wf, kv.astype(BF))
    for cp in cp_w[1:]:
        cp.start()

    def freq(ft, carry):
        r0 = pl.multiple_of(ft * 16, 16)
        for j in range(NJ):
            lanes = slice(128 * j, 128 * (j + 1))
            for a in range(NC):
                yr = yi = None
                for b in range(a + 1):
                    kr = kf[a - b, pl.ds(r0, 8), lanes]
                    ki = kf[a - b, pl.ds(r0 + 8, 8), lanes]
                    ur = uf[b, pl.ds(r0, 8), lanes]
                    ui = uf[b, pl.ds(r0 + 8, 8), lanes]
                    pr = kr * ur - ki * ui
                    pi = kr * ui + ki * ur
                    yr = pr if yr is None else yr + pr
                    yi = pi if yi is None else yi + pi
                yf[a, pl.ds(r0, 16), lanes] = jnp.concatenate([yr, yi], axis=0).astype(BF)
        return carry
    jax.lax.fori_loop(0, C // 8, freq, 0)

    cp_wm.wait()
    cc = c_ref[...].astype(F32)
    cc = cc * jax.nn.sigmoid(cc)
    mod = _dot(jnp.broadcast_to(cc, (8, D)).astype(BF), wm_v[...])[0:1]
    sa, ca, ga, sb, cb, gb = [mod[:, D * i:D * (i + 1)] for i in range(6)]

    cp_q.wait()
    cp_w[0].wait()

    def stage_a(i, carry):
        wi = wi_ref[...]
        y = jnp.concatenate([_dot(wi, yf[i * (TM // C) + t]) for t in range(TM // C)], axis=0)
        r0 = pl.multiple_of(i * TM, TM)
        x = q_v[pl.ds(r0, TM), :].astype(F32)
        h = _ln(x) * (1.0 + ca) + sa
        x2 = x + ga * (h * y)
        hb = _ln(x2) * (1.0 + cb) + sb
        x2_v[pl.ds(r0, TM), :] = x2
        hb_v[pl.ds(r0, TM), :] = hb
        hh_v[pl.ds(r0 + 8, TM), :] = _gelu(_dot(_ln(hb).astype(BF), w1_v[...]))
        return carry
    jax.lax.fori_loop(0, NT, stage_a, 0)

    for cp in cp_w[1:]:
        cp.wait()

    def stage_b(i, carry):
        r0 = pl.multiple_of(i * TM, TM)
        hh = hh_v[pl.ds(r0, TM + 16), :]
        lane = jax.lax.broadcasted_iota(jnp.int32, (TM, 128), 1)
        def sh(d, j):
            return hh[8 + d:8 + d + TM, 128 * j:128 * (j + 1)]
        g = jnp.concatenate([
            sh(-1, 0),
            jnp.where(lane < 32, sh(-1, 1), sh(1, 1)),
            jnp.where(lane < 64, sh(1, 2), sh(-2, 2)),
            jnp.where(lane < 96, sh(-2, 3), sh(2, 3)),
            sh(2, 4)], axis=1).astype(BF)
        x1 = hb_v[pl.ds(r0, TM), :] + _dot(g, w2_v[...])
        h3 = _gelu(_dot_nt(_ln(x1).astype(BF), w3_v[...])).astype(BF)
        h2 = _dot(h3, w4_v[...])
        out = x2_v[pl.ds(r0, TM), :] + gb * (x1 + h2)
        o_v[pl.ds(r0, TM), :] = out.astype(BF)
        pltpu.make_async_copy(o_v.at[pl.ds(r0, TM)], o_h.at[0, pl.ds(r0, TM)], sems.at[19]).start()
        return carry
    jax.lax.fori_loop(0, NT, stage_b, 0)
    pltpu.make_async_copy(o_v, o_h.at[0], sems.at[19]).wait()


@jax.jit
def pallas_adaLN_cond__ssm_conv_h3__mixer_s_mlp__prompt_kernel(
    A_q, A_k, A_v, A_shift_k, A_ssm_k, A_ssm_D, B_x, B_w1, B_w2, B_w3, B_w4, c, w_mod,
):
    hbm = pl.BlockSpec(memory_space=pltpu.MemorySpace.HBM)
    return pl.pallas_call(
        _kernel,
        in_specs=[hbm] * 14,
        out_specs=hbm,
        out_shape=jax.ShapeDtypeStruct((1, S, D), BF),
        scratch_shapes=[
            pltpu.VMEM((4, D), BF), pltpu.VMEM((D,), BF), pltpu.VMEM((1, D), BF),
            pltpu.VMEM((2 * C, C), BF), pltpu.VMEM((C, 2 * C), BF),
            pltpu.VMEM((S, D), BF), pltpu.VMEM((S + 16, D), BF), pltpu.VMEM((S, D), BF),
            pltpu.VMEM((D, S), BF), pltpu.VMEM((D, D), BF), pltpu.VMEM((D, D), BF),
            pltpu.VMEM((F, D), BF), pltpu.VMEM((F, D), BF), pltpu.VMEM((D, 6 * D), BF),
            pltpu.VMEM((NC, 2 * C, D), F32), pltpu.VMEM((NC, 2 * C, D), F32),
            pltpu.VMEM((NC, 2 * C, D), BF),
            pltpu.VMEM((S, D), F32), pltpu.VMEM((S, D), F32), pltpu.VMEM((S + 16, D), F32),
            pltpu.VMEM((S, D), BF),
            pltpu.SemaphoreType.DMA((25,)),
        ],
        compiler_params=pltpu.CompilerParams(vmem_limit_bytes=110 * 1024 * 1024),
    )(A_q, A_k, A_v, A_shift_k.T, A_ssm_k, A_ssm_D, B_w1, B_w2, B_w3.T, B_w4, c, w_mod, _WF, _WI)
```

```python
import numpy as np
import jax
import jax.numpy as jnp
import jax.experimental.pallas as pl
import jax.experimental.pallas.tpu as pltpu

S, D, F = 2048, 640, 1728
C = 128
NC = S // C
TM = 256
NT = S // TM
EPS = 1e-5
BF, F32 = jnp.bfloat16, jnp.float32


def _dft_mats():
    f = np.concatenate([np.arange(0, C, 2), np.arange(1, C, 2)])
    n = np.arange(C)
    ang = np.pi * (2 * f[:, None] + 1) * n[None, :] / (2 * C)
    re, im = np.cos(ang), -np.sin(ang)
    fwd = np.stack([re.reshape(C // 8, 8, C), im.reshape(C // 8, 8, C)], 1).reshape(2 * C, C)
    inv = fwd.T / C
    return fwd.astype(BF), inv.astype(BF)


_WF, _WI = _dft_mats()


def _ln(x):
    m = jnp.mean(x, axis=-1, keepdims=True)
    xc = x - m
    v = jnp.mean(xc * xc, axis=-1, keepdims=True)
    return xc * jax.lax.rsqrt(v + EPS)


def _gelu(x):
    c0 = float(np.sqrt(2.0 / np.pi))
    t = jnp.tanh(x * (c0 + (c0 * 0.044715) * (x * x)))
    hx = 0.5 * x
    return hx + hx * t


def _dot(a, b):
    return jnp.dot(a, b, preferred_element_type=F32)


def _dot_nt(a, b):
    return jax.lax.dot_general(a, b, (((1,), (1,)), ((), ())), preferred_element_type=F32)


def _kernel(q_h, k_h, v_h, shk_h, ssm_h, ssd_h, w1_h, w2_h, w3_h, w4_h, c_h, wm_h,
            wf_h, wi_h, o_h, shk_ref, ssd_ref, c_ref, wf_ref, wi_ref,
            q_v, k_v, v_v, ssm_v, w1_v, w2_v, w3_v, w4_v, wm_v,
            kf, uf, yf, x2_v, hb_v, hh_v, o_v, ks_v, z1_v, z3_v, zc_v, sems):
    NJ = D // 128
    cp_ssm = [pltpu.make_async_copy(ssm_h.at[pl.ds(128 * j, 128)], ssm_v.at[pl.ds(128 * j, 128)], sems.at[j])
              for j in range(NJ)]
    NK = 4
    RK = S // NK
    cp_k = [pltpu.make_async_copy(k_h.at[0, pl.ds(RK * j, RK)], k_v.at[pl.ds(16 + RK * j, RK)], sems.at[5 + j])
            for j in range(NK)]
    cp_v = [pltpu.make_async_copy(v_h.at[0, pl.ds(RK * j, RK)], v_v.at[pl.ds(RK * j, RK)], sems.at[9 + j])
            for j in range(NK)]
    cp_wm = pltpu.make_async_copy(wm_h, wm_v, sems.at[13])
    cp_q = pltpu.make_async_copy(q_h.at[0], q_v, sems.at[14])
    cp_w = [pltpu.make_async_copy(a, b, sems.at[15 + i])
            for i, (a, b) in enumerate([(w1_h, w1_v), (w2_h, w2_v), (w3_h, w3_v), (w4_h, w4_v)])]
    cp_s = [pltpu.make_async_copy(a, b, sems.at[20 + i])
            for i, (a, b) in enumerate([(wf_h, wf_ref), (ssd_h, ssd_ref), (shk_h, shk_ref), (c_h, c_ref), (wi_h, wi_ref)])]
    for cp in cp_s:
        cp.start()
    for cp in cp_ssm:
        cp.start()
    cp_k[0].start()
    cp_v[0].start()

    k_v[pl.ds(0, 16), :] = jnp.zeros((16, D), BF)
    hh_v[pl.ds(0, 8), :] = jnp.zeros((8, D), F32)
    hh_v[pl.ds(8 + S, 8), :] = jnp.zeros((8, D), F32)
    for cp in cp_s:
        cp.wait()
    wf = wf_ref[...]
    ssd = ssd_ref[...].astype(F32).reshape(1, D)

    for j in range(NJ):
        cp_ssm[j].wait()
        if j + 1 < NK:
            cp_k[j + 1].start()
            cp_v[j + 1].start()
        if j == NJ - 2:
            cp_wm.start()
        lanes = slice(128 * j, 128 * (j + 1))
        prev = None
        for m in range(NC):
            kh = _dot_nt(wf, ssm_v[lanes, C * m:C * (m + 1)]).reshape(2, C // 16, 2, 8, 128)
            re, im = kh[:, :, 0], kh[:, :, 1]
            if m == 0:
                re = re + ssd[:, lanes]
                ore, oim = re, im
            else:
                pre, pim = prev
                ore = jnp.stack([re[0] - pim[0], re[1] + pim[1]])
                oim = jnp.stack([im[0] + pre[0], im[1] - pre[1]])
            prev = (re, im)
            kf[m, :, lanes] = jnp.stack([ore, oim], axis=2).reshape(2 * C, 128)

    shk = shk_ref[...].astype(F32)
    for b in range(NC):
        if b % (NC // NK) == 0:
            cp_k[b // (NC // NK)].wait()
            cp_v[b // (NC // NK)].wait()
        if b == 0:
            cp_q.start()
            cp_w[0].start()
        if b == 8:
            for cp in cp_w[1:]:
                cp.start()
        kk = k_v[pl.ds(C * b, C + 16), :].astype(F32)
        ks = kk[16:16 + C] * shk[0:1]
        for t in range(1, 4):
            ks = ks + kk[16 - t:16 - t + C] * shk[t:t + 1]
        kv = ks * v_v[pl.ds(C * b, C), :].astype(F32)
        uf[b] = _dot(wf, kv.astype(BF))
    def freq(ft, carry):
        r0 = pl.multiple_of(ft * 16, 16)
        for m in range(NC):
            ks_v[m] = kf[m, pl.ds(r0, 8), :] + kf[m, pl.ds(r0 + 8, 8), :]
        for j in range(NJ):
            lanes = slice(128 * j, 128 * (j + 1))
            for a0 in range(0, NC, 4):
                acc = {}
                for b in range(a0 + 4):
                    ur = uf[b, pl.ds(r0, 8), lanes]
                    ui = uf[b, pl.ds(r0 + 8, 8), lanes]
                    us = ur + ui
                    for a in range(max(a0, b), a0 + 4):
                        p = (kf[a - b, pl.ds(r0, 8), lanes] * ur,
                             kf[a - b, pl.ds(r0 + 8, 8), lanes] * ui,
                             ks_v[a - b, :, lanes] * us)
                        acc[a] = p if a not in acc else tuple(x + y for x, y in zip(acc[a], p))
                for a, (t1, t2, t3) in acc.items():
                    yf[a, pl.ds(r0, 16), lanes] = jnp.concatenate([t1 - t2, t3 - t1 - t2], axis=0).astype(BF)
        return carry
    jax.lax.fori_loop(0, C // 8, freq, 0)

    cp_wm.wait()
    cc = c_ref[...].astype(F32)
    cc = cc * jax.nn.sigmoid(cc)
    mod = _dot(jnp.broadcast_to(cc, (8, D)).astype(BF), wm_v[...])[0:1]
    sa, ca, ga, sb, cb, gb = [mod[:, D * i:D * (i + 1)] for i in range(6)]

    cp_q.wait()
    cp_w[0].wait()

    def gate(ch):
        y = _dot(wi_ref[...], yf[ch])
        for r in range(0, C, 64):
            rows = pl.ds(pl.multiple_of(ch * C + r, 64), 64)
            x = q_v[rows, :].astype(F32)
            h = _ln(x) * (1.0 + ca) + sa
            x2 = x + ga * (h * y[r:r + 64])
            hb = _ln(x2) * (1.0 + cb) + sb
            x2_v[rows, :] = x2
            hb_v[rows, :] = hb
            z1_v[pl.ds(pl.multiple_of((ch % 2) * C + r, 64), 64), :] = _ln(hb).astype(BF)

    def mix_in(i):
        hh_v[pl.ds(pl.multiple_of(i * TM, TM) + 8, TM), :] = _gelu(_dot(z1_v[...], w1_v[...]))

    def mix_out(i, half):
        r0 = pl.multiple_of(i * TM + half * C, C)
        hh = hh_v[pl.ds(r0, C + 16), :]
        lane = jax.lax.broadcasted_iota(jnp.int32, (C, 128), 1)
        def sh(d, j):
            return hh[8 + d:8 + d + C, 128 * j:128 * (j + 1)]
        g = jnp.concatenate([
            sh(-1, 0),
            jnp.where(lane < 32, sh(-1, 1), sh(1, 1)),
            jnp.where(lane < 64, sh(1, 2), sh(-2, 2)),
            jnp.where(lane < 96, sh(-2, 3), sh(2, 3)),
            sh(2, 4)], axis=1).astype(BF)
        x1 = hb_v[pl.ds(r0, C), :] + _dot(g, w2_v[...])
        hb_v[pl.ds(r0, C), :] = x1
        z3_v[pl.ds(half * C, C), :] = _ln(x1).astype(BF)

    def mlp(i, side):
        r0 = pl.multiple_of(i * TM, TM)
        zc_v[...] = z3_v[...]
        acc = None
        for n, f0 in enumerate(range(0, F, 256)):
            fs = slice(f0, min(f0 + 256, F))
            h3 = _gelu(_dot_nt(zc_v[...], w3_v[fs, :])).astype(BF)
            p = _dot(h3, w4_v[fs, :])
            acc = p if acc is None else acc + p
            if n < len(side):
                side[n]()
        out = x2_v[pl.ds(r0, TM), :] + gb * (hb_v[pl.ds(r0, TM), :] + acc)
        o_v[pl.ds(r0, TM), :] = out.astype(BF)
        pltpu.make_async_copy(o_v.at[pl.ds(r0, TM)], o_h.at[0, pl.ds(r0, TM)], sems.at[19]).start()

    def head(i, carry):
        gate(2 * i)
        gate(2 * i + 1)
        mix_in(i)
        return carry
    jax.lax.fori_loop(0, 2, head, 0)
    cp_w[1].wait()
    mix_out(0, 0)
    mix_out(0, 1)
    cp_w[2].wait()
    cp_w[3].wait()

    def steady(i, carry):
        mlp(i, [lambda: gate(2 * i + 4), lambda: gate(2 * i + 5), lambda: mix_out(i + 1, 0),
                lambda: mix_in(i + 2), lambda: mix_out(i + 1, 1)])
        return carry
    jax.lax.fori_loop(0, NT - 2, steady, 0)
    mlp(NT - 2, [lambda: mix_out(NT - 1, 0), lambda: mix_out(NT - 1, 1)])
    mlp(NT - 1, [])
    pltpu.make_async_copy(o_v, o_h.at[0], sems.at[19]).wait()


@jax.jit
def pallas_adaLN_cond__ssm_conv_h3__mixer_s_mlp__prompt_kernel(
    A_q, A_k, A_v, A_shift_k, A_ssm_k, A_ssm_D, B_x, B_w1, B_w2, B_w3, B_w4, c, w_mod,
):
    hbm = pl.BlockSpec(memory_space=pltpu.MemorySpace.HBM)
    return pl.pallas_call(
        _kernel,
        in_specs=[hbm] * 14,
        out_specs=hbm,
        out_shape=jax.ShapeDtypeStruct((1, S, D), BF),
        scratch_shapes=[
            pltpu.VMEM((4, D), BF), pltpu.VMEM((D,), BF), pltpu.VMEM((1, D), BF),
            pltpu.VMEM((2 * C, C), BF), pltpu.VMEM((C, 2 * C), BF),
            pltpu.VMEM((S, D), BF), pltpu.VMEM((S + 16, D), BF), pltpu.VMEM((S, D), BF),
            pltpu.VMEM((D, S), BF), pltpu.VMEM((D, D), BF), pltpu.VMEM((D, D), BF),
            pltpu.VMEM((F, D), BF), pltpu.VMEM((F, D), BF), pltpu.VMEM((D, 6 * D), BF),
            pltpu.VMEM((NC, 2 * C, D), F32), pltpu.VMEM((NC, 2 * C, D), F32),
            pltpu.VMEM((NC, 2 * C, D), BF),
            pltpu.VMEM((S, D), F32), pltpu.VMEM((S, D), F32), pltpu.VMEM((S + 16, D), F32),
            pltpu.VMEM((S, D), BF),
            pltpu.VMEM((NC, 8, D), F32),
            pltpu.VMEM((TM, D), BF), pltpu.VMEM((TM, D), BF), pltpu.VMEM((TM, D), BF),
            pltpu.SemaphoreType.DMA((25,)),
        ],
        compiler_params=pltpu.CompilerParams(vmem_limit_bytes=110 * 1024 * 1024),
    )(A_q, A_k, A_v, A_shift_k.T, A_ssm_k, A_ssm_D, B_w1, B_w2, B_w3.T, B_w4, c, w_mod, _WF, _WI)
```
